```python
import jax
import jax.numpy as jnp

def _softmax(x, axis=-1):
    return jax.nn.softmax(x, axis=axis)
def _gelu(x):
    return jax.nn.gelu(x, approximate=True)
def _silu(x):
    return jax.nn.silu(x)
def _sigmoid(x):
    return jax.nn.sigmoid(x)
def _layernorm(x, axis=-1, eps=1e-5):
    m = jnp.mean(x, axis=axis, keepdims=True)
    v = jnp.var(x, axis=axis, keepdims=True)
    return (x - m) / jnp.sqrt(v + eps)
def _scatter_add(tgt, idx, src, axis=0):
    return tgt.at[idx].add(src)
def _segment_sum(src, seg, n):
    return jax.ops.segment_sum(src, seg, n)
class _Rng:
    def __init__(self, key):
        self._k = key
    def _next(self):
        self._k, sub = jax.random.split(self._k)
        return sub
    def normal(self, shape):
        return jax.random.normal(self._next(), shape, dtype=jnp.bfloat16)
    def randint(self, lo, hi, shape):
        return jax.random.randint(self._next(), shape, lo, hi, dtype=jnp.int32)
    def uniform(self, shape, lo=0.0, hi=1.0):
        return jax.random.uniform(self._next(), shape, jnp.bfloat16, lo, hi)
    def permutation(self, n):
        return jax.random.permutation(self._next(), n)


kernel_name = 'gated_mix__compressed_kv_cla__sliding_local_dilated__prompt'

def setup_inputs():
    _rng = _Rng(jax.random.key(int.from_bytes(__import__("os").urandom(4), "little")))
    _w = (lambda a: (lambda t: t.astype(jnp.bfloat16) if jnp.issubdtype(t.dtype, jnp.floating) else t)(jnp.asarray(a)))
    def _A_setup():
        B, H, Sq, Sk, D, M = 1, 32, 2048, 2048, 128, 1024
        Dc = 4 * D
        return {
            "x": _w((lambda *s: _rng.normal(s) * 0.05)(B, Sq, M)),
            "c_kv": _w((lambda *s: _rng.normal(s) * 0.05)(B, Sk, Dc)),
            "w_q": _w((lambda *s: _rng.normal(s) * 0.05)(M, H, D) * (M ** -0.5)),
            "w_uk": _w((lambda *s: _rng.normal(s) * 0.05)(Dc, H, D) * (Dc ** -0.5)),
            "w_uv": _w((lambda *s: _rng.normal(s) * 0.05)(Dc, H, D) * (Dc ** -0.5)),
            "w_o": _w((lambda *s: _rng.normal(s) * 0.05)(H, D, M) * ((H * D) ** -0.5)),
        }
    _A_in = _A_setup()

    def _B_setup():
        B, S, D = 1, 2048, 1024
        return {
            "x": _w((lambda *s: _rng.normal(s) * 0.05)(B, S, D)),
            "wqkv": _w((lambda *s: _rng.normal(s) * 0.05)(D, 3 * D)),
            "wo": _w((lambda *s: _rng.normal(s) * 0.05)(D, D)),
        }
    _B_in = _B_setup()

    return {
        "A_x": _A_in["x"],
        "A_c_kv": _A_in["c_kv"],
        "A_w_q": _A_in["w_q"],
        "A_w_uk": _A_in["w_uk"],
        "A_w_uv": _A_in["w_uv"],
        "A_w_o": _A_in["w_o"],
        "B_x": _B_in["x"],
        "B_wqkv": _B_in["wqkv"],
        "B_wo": _B_in["wo"],
        "gate_w": _w((lambda *s: _rng.normal(s) * 0.05)(1024)),
    }

def reference(A_x, A_c_kv, A_w_q, A_w_uk, A_w_uv, A_w_o, B_x, B_wqkv, B_wo, gate_w):
    def _A_ref(x, c_kv, w_q, w_uk, w_uv, w_o):
        B, Sq, M = x.shape[0], x.shape[1], x.shape[2]
        Sk = c_kv.shape[1]
        H, D = w_q.shape[1], w_q.shape[2]
        q = jnp.einsum("bqm,mhd->bhqd", x, w_q)
        k = jnp.einsum("bkc,chd->bhkd", c_kv, w_uk)
        v = jnp.einsum("bkc,chd->bhkd", c_kv, w_uv)
        scores = jnp.einsum("bhqd,bhkd->bhqk", q, k) * (D ** -0.5)
        off = Sk - Sq
        qi = jnp.arange(Sq)[:, None]
        kj = jnp.arange(Sk)[None, :]
        cmask = kj <= (qi + off)
        scores = jnp.where(cmask[None, None], scores, -1e9)
        p = _softmax(scores, axis=-1)
        ctx = jnp.einsum("bhqk,bhkd->bhqd", p, v)
        return jnp.einsum("bhqd,hdm->bqm", ctx, w_o)

    def _B_ref(x, wqkv, wo):
        B, S, D = x.shape
        H = 32; Dh = D // H
        W, dil = 8, 2
        qkv = (lambda x, *d: x.transpose(*d))((x @ wqkv).reshape(B, S, 3, H, Dh), 2, 0, 3, 1, 4)
        q, k, v = qkv[0], qkv[1], qkv[2]
        scale = Dh ** -0.5
        pos = jnp.arange(S)
        off = jnp.arange(W) * dil
        idx = pos[:, None] - off[None, :]
        mask = idx >= 0
        idx_c = jnp.where(mask, idx, 0).reshape(-1)
        kg = k[:, :, idx_c, :].reshape(B, H, S, W, Dh)
        vg = v[:, :, idx_c, :].reshape(B, H, S, W, Dh)
        logits = jnp.einsum("bhsd,bhswd->bhsw", q, kg) * scale
        logits = jnp.where(mask[None, None, :, :], logits, -1e9)
        attn = _softmax(logits, axis=-1)
        o = jnp.einsum("bhsw,bhswd->bhsd", attn, vg)
        return (lambda x, *d: x.transpose(*d))(o, 0, 2, 1, 3).reshape(B, S, D) @ wo

    x = A_x
    g = _sigmoid((x * gate_w).sum(-1, keepdims=True))
    a = _A_ref(x, A_c_kv, A_w_q, A_w_uk, A_w_uv, A_w_o)
    b = _B_ref(x, B_wqkv, B_wo)
    return g * a + (1 - g) * b
```

```python
import functools
import math
import os as _os

import jax
import jax.numpy as jnp
from jax import lax
import jax.experimental.pallas as pl
import jax.experimental.pallas.tpu as pltpu

S = 2048
M = 1024
H = 32
D = 128
DC = 512
DH = 32
W_B = 8
DIL = 2
KCAT = H * D + M

BQ = int(_os.environ.get("K_BQ", "256"))
TK = int(_os.environ.get("K_TK", "256"))
PIPE = int(_os.environ.get("K_PIPE", "1"))
PCH = int(_os.environ.get("K_PCH", "4"))
TLAG = int(_os.environ.get("K_TLAG", "2"))
FJ = int(_os.environ.get("K_FJ", "1"))
BSTEP = int(_os.environ.get("K_BSTEP", "4"))
HG = 8
CH = S // HG
OUT_ROWS = int(_os.environ.get("K_OR", "256"))
N_OUT = S // OUT_ROWS
LOG2E = math.log2(math.e)
NEG = -1e9

_NT = (((1,), (1,)), ((), ()))
_TT = (((0,), (1,)), ((), ()))


def _attn_a(q_ref, k_ref, v_ref, g_ref, cat_ref, hcol, never, tie0):
    nq = S // BQ
    row = lax.broadcasted_iota(jnp.int32, (BQ, BQ), 0)
    col = lax.broadcasted_iota(jnp.int32, (BQ, BQ), 1)
    causal = col <= row

    def tiles(i):
        lo = i * BQ
        t = [(s0, min(TK, lo - s0), False) for s0 in range(0, lo, TK)]
        return t + [(lo, BQ, True)]

    def qk(i, t):
        s0, w, diag = t
        s = lax.dot_general(q_ref[pl.ds(i * BQ, BQ), :], k_ref[pl.ds(s0, w), :], _NT,
                            preferred_element_type=jnp.float32)
        return jnp.where(causal, s, NEG) if diag else s

    def fold(s, op):
        parts = [s[:, c0:c0 + 128] for c0 in range(0, s.shape[1], 128)]
        return functools.reduce(op, parts)

    def qk_block(i):
        ss, mx = [], None
        for t in tiles(i):
            s = qk(i, t)
            ss.append(s)
            f = fold(s, jnp.maximum)
            mx = f if mx is None else jnp.maximum(mx, f)
            yield
        yield ss, jnp.max(mx, axis=1, keepdims=True)

    finals = {-k: tie0 for k in range(1, TLAG + 1)}

    def pv_block(i, ss, m):
        lsum, o = None, None
        m = jnp.where(never, finals[i - TLAG], jnp.broadcast_to(m, (BQ, 128)))
        for t, s in zip(tiles(i), ss):
            p = jnp.exp2(s - jnp.concatenate([m] * (t[1] // 128), axis=1))
            f = fold(p, jnp.add)
            lsum = f if lsum is None else lsum + f
            d = jnp.dot(p.astype(jnp.bfloat16), v_ref[pl.ds(t[0], t[1]), :],
                        preferred_element_type=jnp.float32)
            o = d if o is None else o + d
            yield
        l = jnp.sum(lsum, axis=1, keepdims=True)
        r = pl.reciprocal(l, approx=True)
        r = r * (2.0 - l * r)
        o = o * (g_ref[pl.ds(i * BQ, BQ), :] * r)
        finals[i] = o
        cat_ref[pl.ds(i * BQ, BQ), pl.ds(hcol, D)] = o.astype(jnp.bfloat16)

    def drain(gen):
        r = None
        for r in gen:
            pass
        return r

    if not PIPE:
        for i in range(nq):
            ss, m = drain(qk_block(i))
            drain(pv_block(i, ss, m))
        return
    cur = drain(qk_block(0))
    for i in range(nq):
        pv = pv_block(i, *cur)
        if i + 1 < nq:
            nxt = qk_block(i + 1)
            r = next(nxt)
            while r is None:
                next(pv, None)
                r = next(nxt)
            cur = r
        drain(pv)


def _attn_b(bt_ref, g_ref, cat_ref, step, ties):
    c0 = pl.multiple_of((step % HG) * CH, CH)
    pos = c0 + lax.broadcasted_iota(jnp.int32, (HG, CH), 1)

    def taps(j, d):
        win = bt_ref[j, d, :, pl.ds(c0, CH + 128)]
        return [win[:, 128:] if w == 0 else pltpu.roll(win, w * DIL, 1)[:, 128:]
                for w in range(W_B)]

    logits = [None] * W_B
    for d in range(DH):
        qd = bt_ref[0, d, :, pl.ds(c0 + 128, CH)]
        for w, kw in enumerate(taps(1, d)):
            logits[w] = qd * kw if d == 0 else logits[w] + qd * kw
        yield
    logits = [l * (LOG2E * DH ** -0.5) for l in logits]
    logits = [l if w == 0 else jnp.where(pos >= w * DIL, l, NEG) for w, l in enumerate(logits)]
    mb = functools.reduce(jnp.maximum, logits)
    ps = [jnp.exp2(l - mb) for l in logits]
    inv = 1.0 / functools.reduce(lambda a, b: a + b, ps)
    ps = [p * inv for p in ps]
    yield
    outs = []
    for d in range(DH):
        acc = None
        for w, vw in enumerate(taps(2, d)):
            acc = ps[w] * vw if w == 0 else acc + ps[w] * vw
        outs.append(acc)
        yield
    o = jnp.swapaxes(jnp.stack(outs, 0), 0, 1).reshape(HG * DH, CH)
    gi = 1.0 - g_ref[pl.ds(c0, CH), :]
    bcol = pl.multiple_of(H * D + (step // HG) * (HG * DH), HG * DH)
    for j in range(HG * DH // 128):
        oj = o[j * 128:(j + 1) * 128, :].T * gi
        cat_ref[pl.ds(c0, CH), pl.ds(bcol + j * 128, 128)] = oj.astype(jnp.bfloat16)
        ties.append(oj[0:8] + oj[CH - 8:CH])
    yield


def _kernel(x_ref, c_ref, wq_ref, wuk_ref, wuv_ref, wbq_ref, wbk_ref, wbv_ref,
            gw_ref, wo_hbm, wob_hbm, out_ref,
            cat_ref, wcat_ref, g_ref, q_ref, k_ref, v_ref, bt_ref,
            wq_s, wuk_s, wuv_s, sem):
    step = pl.program_id(0)

    def wo_copies():
        return (
            pltpu.make_async_copy(wo_hbm, wcat_ref.at[pl.ds(0, H * D), :], sem.at[0]),
            pltpu.make_async_copy(wob_hbm, wcat_ref.at[pl.ds(H * D, M), :], sem.at[1]),
        )

    @pl.when(step == 0)
    def _():
        for cp in wo_copies():
            cp.start()
        bt_ref[:, :, :, pl.ds(0, 128)] = jnp.zeros((3, DH, HG, 128), jnp.float32)
        gw = jnp.broadcast_to(gw_ref[...], (16, M))
        z = lax.dot_general(gw, x_ref[...], _NT, preferred_element_type=jnp.float32)
        g = jax.nn.sigmoid(z[0:8])
        g = jnp.concatenate([g] * 16, axis=0)
        for r in range(S // 128):
            g_ref[pl.ds(r * 128, 128), :] = g[:, r * 128:(r + 1) * 128].T

    @pl.when(jnp.logical_and(step < H, step % HG == 0))
    def _():
        wq_s[...] = jnp.swapaxes(wq_ref[...], 0, 1)
        wuk_s[...] = jnp.swapaxes(wuk_ref[...], 0, 1)
        wuv_s[...] = jnp.swapaxes(wuv_ref[...], 0, 1)
        x = x_ref[...]
        for j, w_ref in enumerate((wbq_ref, wbk_ref, wbv_ref)):
            t = lax.dot_general(w_ref[...], x, _TT, preferred_element_type=jnp.float32)
            bt_ref[j, :, :, pl.ds(128, S)] = jnp.swapaxes(t.reshape(HG, DH, S), 0, 1)

    @pl.when(step < H)
    def _():
        h = step
        hl = h % HG
        ties = []
        bgen = _attn_b(bt_ref, g_ref, cat_ref, step, ties)
        c = c_ref[...]
        npc = PCH
        rows = S // npc
        for r in range(npc):
            k_ref[pl.ds(r * rows, rows), :] = jnp.dot(
                c[r * rows:(r + 1) * rows], wuk_s[hl], preferred_element_type=jnp.float32
            ).astype(jnp.bfloat16)
            for _ in range(BSTEP):
                next(bgen, None)
        for r in range(npc):
            q_ref[pl.ds(r * rows, rows), :] = (jnp.dot(
                x_ref[pl.ds(r * rows, rows), :], wq_s[hl], preferred_element_type=jnp.float32)
                * (LOG2E * D ** -0.5)).astype(jnp.bfloat16)
            for _ in range(2 * BSTEP):
                next(bgen, None)
        for r in range(npc):
            v_ref[pl.ds(r * rows, rows), :] = jnp.dot(
                c[r * rows:(r + 1) * rows], wuv_s[hl], preferred_element_type=jnp.float32
            ).astype(jnp.bfloat16)
            for _ in range(BSTEP):
                next(bgen, None)
        for _ in bgen:
            pass
        tie = functools.reduce(jnp.add, ties)
        tie = jnp.concatenate([tie] * (BQ // 8), 0)
        _attn_a(q_ref, k_ref, v_ref, g_ref, cat_ref, pl.multiple_of(h * D, D), step < 0, tie)

    @pl.when(step == H)
    def _():
        for cp in wo_copies():
            cp.wait()

    @pl.when(step >= H)
    def _():
        r = pl.multiple_of((step - H) * OUT_ROWS, OUT_ROWS)
        out_ref[...] = jnp.dot(cat_ref[pl.ds(r, OUT_ROWS), :], wcat_ref[...],
                               preferred_element_type=jnp.float32).astype(out_ref.dtype)


@jax.jit
def pallas_gated_mix__compressed_kv_cla__sliding_local_dilated__prompt_kernel(
    A_x: jax.Array,
    A_c_kv: jax.Array,
    A_w_q: jax.Array,
    A_w_uk: jax.Array,
    A_w_uv: jax.Array,
    A_w_o: jax.Array,
    B_x: jax.Array,
    B_wqkv: jax.Array,
    B_wo: jax.Array,
    gate_w: jax.Array,
):
    del B_x
    x = A_x.reshape(S, M)
    c = A_c_kv.reshape(S, DC)
    wo = A_w_o.reshape(H * D, M)
    gw = gate_w.reshape(1, M)

    def hd(s):
        return jnp.minimum(s, H - 1)

    nb = M // (HG * DH)
    out = pl.pallas_call(
        _kernel,
        grid=(H + N_OUT,),
        in_specs=[
            pl.BlockSpec((S, M), lambda s: (0, 0)),
            pl.BlockSpec((S, DC), lambda s: (0, 0)),
            pl.BlockSpec((M, HG, D), lambda s: (0, hd(s) // HG, 0)),
            pl.BlockSpec((DC, HG, D), lambda s: (0, hd(s) // HG, 0)),
            pl.BlockSpec((DC, HG, D), lambda s: (0, hd(s) // HG, 0)),
            pl.BlockSpec((M, HG * DH), lambda s: (0, hd(s) // HG)),
            pl.BlockSpec((M, HG * DH), lambda s: (0, nb + hd(s) // HG)),
            pl.BlockSpec((M, HG * DH), lambda s: (0, 2 * nb + hd(s) // HG)),
            pl.BlockSpec((1, M), lambda s: (0, 0)),
            pl.BlockSpec(memory_space=pl.ANY),
            pl.BlockSpec(memory_space=pl.ANY),
        ],
        out_specs=pl.BlockSpec((OUT_ROWS, M), lambda s: (jnp.maximum(s - H, 0), 0)),
        out_shape=jax.ShapeDtypeStruct((S, M), jnp.bfloat16),
        scratch_shapes=[
            pltpu.VMEM((S, KCAT), jnp.bfloat16),
            pltpu.VMEM((KCAT, M), jnp.bfloat16),
            pltpu.VMEM((S, 128), jnp.float32),
            pltpu.VMEM((S, D), jnp.bfloat16),
            pltpu.VMEM((S, D), jnp.bfloat16),
            pltpu.VMEM((S, D), jnp.bfloat16),
            pltpu.VMEM((3, DH, HG, 128 + S), jnp.float32),
            pltpu.VMEM((HG, M, D), jnp.bfloat16),
            pltpu.VMEM((HG, DC, D), jnp.bfloat16),
            pltpu.VMEM((HG, DC, D), jnp.bfloat16),
            pltpu.SemaphoreType.DMA((2,)),
        ],
        compiler_params=pltpu.CompilerParams(
            dimension_semantics=("arbitrary",),
            vmem_limit_bytes=100 * 1024 * 1024,
        ),
    )(x, c, A_w_q, A_w_uk, A_w_uv, B_wqkv, B_wqkv, B_wqkv, gw, wo, B_wo)
    return out.reshape(1, S, M)
```

```python
import functools
import math
import os as _os

import jax
import jax.numpy as jnp
from jax import lax
import jax.experimental.pallas as pl
import jax.experimental.pallas.tpu as pltpu

S = 2048
M = 1024
H = 32
D = 128
DC = 512
DH = 32
W_B = 8
DIL = 2
KCAT = H * D + M

BQ = 256
HQ = BQ // 2
TK = int(_os.environ.get("K_TK", "256"))
RP = int(_os.environ.get("K_RP", "32"))
FB = int(_os.environ.get("K_FB", "3"))
BT0 = int(_os.environ.get("K_BT0", "1"))
TLAG = int(_os.environ.get("K_TLAG", "2"))
F0 = int(_os.environ.get("K_F0", "2"))
F1 = int(_os.environ.get("K_F1", "2"))
LEAD = int(_os.environ.get("K_LEAD", "2"))
HG = 8
NG = H // HG
CH = S // HG
NX = 4
XR = S // NX
OUT_ROWS = int(_os.environ.get("K_OR", "128"))
N_OUT = S // OUT_ROWS
LOG2E = math.log2(math.e)
NEG = -1e9

_NT = (((1,), (1,)), ((), ()))
_TT = (((0,), (1,)), ((), ()))


def _drain(gen):
    for _ in gen:
        pass


def _fold(s, op):
    return functools.reduce(op, [s[:, c0:c0 + 128] for c0 in range(0, s.shape[1], 128)])


def _tied(a, tie):
    if tie is None:
        return a
    never, t = tie
    first = jnp.where(never, t[0:16, 0:128].astype(a.dtype), a[0:16, 0:128])
    return jnp.concatenate([jnp.concatenate([first, a[0:16, 128:]], axis=1), a[16:]], axis=0)


def _proj(x_ref, c_ref, wq_s, wuk_s, wuv_s, q_ref, k_ref, v_ref, h, slot):
    tie = yield
    for w_s, o_ref in ((wuk_s, k_ref), (wuv_s, v_ref)):
        for r in range(2):
            rows = pl.ds(r * (S // 2), S // 2)
            o_ref[slot, rows, :] = jnp.dot(_tied(c_ref[rows, :], tie), w_s[h],
                                           preferred_element_type=jnp.float32
                                           ).astype(jnp.bfloat16)
            tie = yield True
    for r in range(4):
        rows = pl.ds(r * (S // 4), S // 4)
        q = jnp.dot(_tied(x_ref[rows, :], tie), wq_s[h], preferred_element_type=jnp.float32)
        q_ref[slot, rows, :] = (q * (LOG2E * D ** -0.5)).astype(jnp.bfloat16)
        tie = yield True


def _attn_a(q_ref, k_ref, v_ref, g_ref, cat_ref, slot, hcol, never, filler, side):
    nq = S // BQ
    row = lax.broadcasted_iota(jnp.int32, (BQ, HQ), 0)
    col = lax.broadcasted_iota(jnp.int32, (BQ, HQ), 1)
    mask_a = col <= row
    mask_b = mask_a[:HQ]
    finals = {}

    def qk_block(i):
        lo = i * BQ
        q = q_ref[slot, pl.ds(lo, BQ), :]
        ss, mx = [], None
        for s0 in range(0, lo, TK):
            s = lax.dot_general(q, k_ref[slot, pl.ds(s0, min(TK, lo - s0)), :], _NT,
                                preferred_element_type=jnp.float32)
            ss.append(s)
            f = _fold(s, jnp.maximum)
            mx = f if mx is None else jnp.maximum(mx, f)
            yield None
        sa = lax.dot_general(q, k_ref[slot, pl.ds(lo, HQ), :], _NT,
                             preferred_element_type=jnp.float32)
        sa = jnp.where(mask_a, sa, NEG)
        sb = lax.dot_general(q[HQ:], k_ref[slot, pl.ds(lo + HQ, HQ), :], _NT,
                             preferred_element_type=jnp.float32)
        sb = jnp.where(mask_b, sb, NEG)
        mx = sa if mx is None else jnp.maximum(mx, sa)
        mx = jnp.concatenate([mx[:HQ], jnp.maximum(mx[HQ:], sb)], axis=0)
        m = jnp.broadcast_to(jnp.max(mx, axis=1, keepdims=True), (BQ, 128))
        yield ss, sa, sb, m

    def pv_block(i, ss, sa, sb, m, last=False):
        lo = i * BQ
        if i - TLAG in finals:
            m = jnp.where(never, finals[i - TLAG], m)
        lsum, o, ps = None, None, []
        for s in ss:
            p = jnp.exp2(s - jnp.concatenate([m] * (s.shape[1] // 128), axis=1))
            f = _fold(p, jnp.add)
            lsum = f if lsum is None else lsum + f
            ps.append(p.astype(jnp.bfloat16))
        if last:
            fill(F1, lsum)
        for t, p in enumerate(ps):
            d = jnp.dot(p, v_ref[slot, pl.ds(t * TK, p.shape[1]), :],
                        preferred_element_type=jnp.float32)
            o = d if o is None else o + d
            yield
        pa = jnp.exp2(sa - m)
        d = jnp.dot(pa.astype(jnp.bfloat16), v_ref[slot, pl.ds(lo, HQ), :],
                    preferred_element_type=jnp.float32)
        o = d if o is None else o + d
        lsum = pa if lsum is None else lsum + pa
        pb = jnp.exp2(sb - m[HQ:])
        d = jnp.dot(pb.astype(jnp.bfloat16), v_ref[slot, pl.ds(lo + HQ, HQ), :],
                    preferred_element_type=jnp.float32)
        o = jnp.concatenate([o[:HQ], o[HQ:] + d], axis=0)
        lsum = jnp.concatenate([lsum[:HQ], lsum[HQ:] + pb], axis=0)
        l = jnp.sum(lsum, axis=1, keepdims=True)
        r = pl.reciprocal(l, approx=True)
        r = r * (2.0 - l * r)
        o = o * (g_ref[pl.ds(lo, BQ), :] * r)
        finals[i] = o
        cat_ref[pl.ds(lo, BQ), pl.ds(hcol, D)] = o.astype(jnp.bfloat16)
        yield

    left = [8 if filler is not None else 0]

    def fill(n, tie=None):
        for k in range(n):
            if left[0] > 0:
                left[0] -= 1
                filler.send((never, tie) if (tie is not None and k == n - 1) else None)

    cur = next(qk_block(0))
    fill(F0)
    for i in range(nq - 1):
        pv, nxt = pv_block(i, *cur), qk_block(i + 1)
        for _ in range(LEAD):
            r = next(nxt)
            if r is not None:
                break
        while r is None:
            next(pv, None)
            r = next(nxt)
        cur = r
        _drain(pv)
    _drain(pv_block(nq - 1, *cur, last=True))
    fill(left[0] - FB)
    tie = next(side)
    fill(1, tie if BT0 else None)
    fill(left[0] - 1)
    fill(1, next(side))


def _attn_b(bt_ref, ot_ref, g_ref, cat_ref, h):
    c0 = pl.multiple_of((h % HG) * CH, CH)
    pos = c0 + lax.broadcasted_iota(jnp.int32, (HG, CH), 1)

    def taps(j, d):
        win = bt_ref[j, d, :, pl.ds(c0, CH + 128)]
        return [win[:, 128:] if w == 0 else pltpu.roll(win, w * DIL, 1)[:, 128:]
                for w in range(W_B)]

    logits = [None] * W_B
    for d in range(DH):
        qd = bt_ref[0, d, :, pl.ds(c0 + 128, CH)]
        for w, kw in enumerate(taps(1, d)):
            logits[w] = qd * kw if d == 0 else logits[w] + qd * kw
    logits = [l * (LOG2E * DH ** -0.5) for l in logits]
    logits = [l if w == 0 else jnp.where(pos >= w * DIL, l, NEG) for w, l in enumerate(logits)]
    mb = functools.reduce(jnp.maximum, logits)
    ps = [jnp.exp2(l - mb) for l in logits]
    inv = 1.0 / functools.reduce(lambda a, b: a + b, ps)
    ps = [p * inv for p in ps]
    tie = functools.reduce(jnp.add, ps)
    yield jnp.concatenate([tie[:, :128], tie[:, 128:]], axis=0)
    for d in range(DH):
        acc = None
        for w, vw in enumerate(taps(2, d)):
            acc = ps[w] * vw if w == 0 else acc + ps[w] * vw
        ot_ref[d] = acc
    o = jnp.swapaxes(ot_ref[...], 0, 1).reshape(HG * DH, CH)
    gi = 1.0 - g_ref[pl.ds(c0, CH), :]
    bcol = pl.multiple_of(H * D + (h // HG) * (HG * DH), HG * DH)
    for j in range(HG * DH // 128):
        oj = o[j * 128:(j + 1) * 128, :].T * gi
        cat_ref[pl.ds(c0, CH), pl.ds(bcol + j * 128, 128)] = oj.astype(jnp.bfloat16)
        tie = oj[0:16] + oj[CH - 16:] if j == 0 else tie + oj[0:16] + oj[CH - 16:]
    yield tie


def _kernel(x_hbm, c_hbm, wq_hbm, wuk_hbm, wuv_hbm, wb_hbm, gw_ref, wo_hbm, wob_hbm, out_hbm,
            x_s, c_s, wq_raw, wuk_raw, wuv_raw, wq_s, wuk_s, wuv_s, wb_s, cat_ref, wcat_ref,
            g_ref, q_ref, k_ref, v_ref, bt_ref, ot_ref, ostage, sem_x, sem_c, sem_a, sem_b, sem_o,
            sem_out):
    def x_copy(i):
        rows = pl.ds(i * XR, XR)
        return pltpu.make_async_copy(x_hbm.at[rows, :], x_s.at[rows, :], sem_x.at[i])

    def c_copy():
        return pltpu.make_async_copy(c_hbm, c_s, sem_c.at[0])

    def a_copies(g):
        hs = pl.ds(g * HG, HG)
        return [pltpu.make_async_copy(src.at[:, hs, :], dst.at[g], sem_a.at[g, j])
                for j, (src, dst) in enumerate(((wq_hbm, wq_raw), (wuk_hbm, wuk_raw),
                                                (wuv_hbm, wuv_raw)))]

    def b_copies(g):
        return [pltpu.make_async_copy(
            wb_hbm.at[:, pl.ds(pl.multiple_of(j * M + g * (HG * DH), HG * DH), HG * DH)],
            wb_s.at[j, g], sem_b.at[g, j]) for j in range(3)]

    def o_copies():
        return [pltpu.make_async_copy(wo_hbm, wcat_ref.at[pl.ds(0, H * D), :], sem_o.at[0]),
                pltpu.make_async_copy(wob_hbm, wcat_ref.at[pl.ds(H * D, M), :], sem_o.at[1])]

    def out_copy(r, slot):
        return pltpu.make_async_copy(
            ostage.at[slot], out_hbm.at[pl.ds(pl.multiple_of(r * OUT_ROWS, OUT_ROWS), OUT_ROWS), :],
            sem_out.at[slot])

    def start(cps):
        for cp in cps:
            cp.start()

    def wait(cps):
        for cp in cps:
            cp.wait()

    def relayout(g, i, n, parts):
        tie = None
        for raw, dst in ((wq_raw, wq_s), (wuk_raw, wuk_s), (wuv_raw, wuv_s)):
            rows = dst.shape[1] // n
            for p in parts:
                lo, hi = [(rows * k // 3) // RP * RP for k in (p, p + 1)]
                for r in range(lo, rows if p == 2 else hi, RP):
                    r0 = pl.multiple_of(i * rows + r, RP)
                    v = jnp.swapaxes(raw[g, pl.ds(r0, RP)], 0, 1)
                    dst[pl.ds(g * HG, HG), pl.ds(r0, RP), :] = v
                    for hh in range(HG):
                        for rr in range(0, RP, 16):
                            u = v[hh, rr:rr + 16]
                            tie = u if tie is None else jnp.maximum(tie, u)
        return tie

    def b_proj(g, first):
        def body(i, carry):
            if first:
                x_copy(i).wait()

                @pl.when(i == 0)
                def _():
                    start([x_copy(j) for j in range(1, NX)])

                @pl.when(i == 1)
                def _():
                    start([c_copy()] + a_copies(0))

                @pl.when(i == 2)
                def _():
                    start(a_copies(1) + b_copies(1))
            x = x_s[pl.ds(pl.multiple_of(i * XR, XR), XR), :]
            for j in range(3):
                xj = x
                if not first and j > 0:
                    tie = relayout(jnp.minimum(g + 1, NG - 1), i, NX, (j - 1,))
                    xj = jnp.concatenate([
                        jnp.concatenate([jnp.where(i < 0, tie, x[0:16, 0:128]), x[0:16, 128:]], 1),
                        x[16:]], 0)
                t = lax.dot_general(wb_s[j, g], xj, _TT, preferred_element_type=jnp.float32)
                bt_ref[j, :, :, pl.ds(pl.multiple_of(128 + i * XR, 128), XR)] = jnp.swapaxes(
                    t.reshape(HG, DH, XR), 0, 1)
            if not first:
                relayout(jnp.minimum(g + 1, NG - 1), i, NX, (2,))
            return carry
        lax.fori_loop(0, NX, body, 0)

    x_copy(0).start()
    start(b_copies(0))
    bt_ref[:, :, :, pl.ds(0, 128)] = jnp.zeros((3, DH, HG, 128), jnp.float32)
    wait(b_copies(0))
    b_proj(0, True)
    gw = jnp.broadcast_to(gw_ref[...], (16, M))
    z = lax.dot_general(gw, x_s[...], _NT, preferred_element_type=jnp.float32)
    gt = jax.nn.sigmoid(z[0:8])
    gt = jnp.concatenate([gt] * 16, axis=0)
    for r in range(S // 128):
        g_ref[pl.ds(r * 128, 128), :] = gt[:, r * 128:(r + 1) * 128].T
    wait([c_copy()] + a_copies(0))
    relayout(0, 0, 1, (0, 1, 2))
    wait(a_copies(1))
    relayout(1, 0, 1, (0, 1, 2))
    start(o_copies())
    _drain(_proj(x_s, c_s, wq_s, wuk_s, wuv_s, q_ref, k_ref, v_ref, 0, 0))

    def head(h, nxt):
        never = h < 0
        slot = h % 2
        side = _attn_b(bt_ref, ot_ref, g_ref, cat_ref, h)
        filler = None
        if nxt:
            filler = _proj(x_s, c_s, wq_s, wuk_s, wuv_s, q_ref, k_ref, v_ref, h + 1, 1 - slot)
            next(filler)
        _attn_a(q_ref, k_ref, v_ref, g_ref, cat_ref, slot, pl.multiple_of(h * D, D),
                never, filler, side)
        _drain(side)

    def head_body(h, carry):
        g = h // HG

        @pl.when(jnp.logical_and(h % HG == 0, h > 0))
        def _():
            wait(b_copies(g))

            @pl.when(g + 1 < NG)
            def _():
                wait(a_copies(g + 1))
            b_proj(g, False)

        @pl.when(jnp.logical_and(h % HG == 1, g + 2 < NG))
        def _():
            start(a_copies(g + 2))

        @pl.when(jnp.logical_and(h % HG == 3, g + 1 < NG))
        def _():
            @pl.when(g > 0)
            def _():
                start(b_copies(g + 1))
        head(h, True)
        return carry

    lax.fori_loop(0, H - 1, head_body, 0)
    head(pl.program_id(0) + (H - 1), False)

    wait(o_copies())

    def out_body(r, carry):
        slot = r % 2

        @pl.when(r >= 2)
        def _():
            out_copy(r - 2, slot).wait()
        rows = pl.ds(pl.multiple_of(r * OUT_ROWS, OUT_ROWS), OUT_ROWS)
        ostage[slot] = jnp.dot(cat_ref[rows, :], wcat_ref[...],
                               preferred_element_type=jnp.float32).astype(ostage.dtype)
        out_copy(r, slot).start()
        return carry

    lax.fori_loop(0, N_OUT, out_body, 0)
    out_copy(N_OUT - 2, 0).wait()
    out_copy(N_OUT - 1, 1).wait()


@jax.jit
def pallas_gated_mix__compressed_kv_cla__sliding_local_dilated__prompt_kernel(
    A_x: jax.Array,
    A_c_kv: jax.Array,
    A_w_q: jax.Array,
    A_w_uk: jax.Array,
    A_w_uv: jax.Array,
    A_w_o: jax.Array,
    B_x: jax.Array,
    B_wqkv: jax.Array,
    B_wo: jax.Array,
    gate_w: jax.Array,
):
    del B_x
    x = A_x.reshape(S, M)
    c = A_c_kv.reshape(S, DC)
    wo = A_w_o.reshape(H * D, M)
    gw = gate_w.reshape(1, M)
    bf = jnp.bfloat16
    hbm = pl.BlockSpec(memory_space=pl.ANY)
    out = pl.pallas_call(
        _kernel,
        grid=(1,),
        in_specs=[hbm, hbm, hbm, hbm, hbm, hbm,
                  pl.BlockSpec((1, M), lambda s: (0, 0)), hbm, hbm],
        out_specs=hbm,
        out_shape=jax.ShapeDtypeStruct((S, M), bf),
        scratch_shapes=[
            pltpu.VMEM((S, M), bf),
            pltpu.VMEM((S, DC), bf),
            pltpu.VMEM((NG, M, HG, D), bf),
            pltpu.VMEM((NG, DC, HG, D), bf),
            pltpu.VMEM((NG, DC, HG, D), bf),
            pltpu.VMEM((H, M, D), bf),
            pltpu.VMEM((H, DC, D), bf),
            pltpu.VMEM((H, DC, D), bf),
            pltpu.VMEM((3, NG, M, HG * DH), bf),
            pltpu.VMEM((S, KCAT), bf),
            pltpu.VMEM((KCAT, M), bf),
            pltpu.VMEM((S, 128), jnp.float32),
            pltpu.VMEM((2, S, D), bf),
            pltpu.VMEM((2, S, D), bf),
            pltpu.VMEM((2, S, D), bf),
            pltpu.VMEM((3, DH, HG, 128 + S), jnp.float32),
            pltpu.VMEM((DH, HG, CH), jnp.float32),
            pltpu.VMEM((2, OUT_ROWS, M), bf),
            pltpu.SemaphoreType.DMA((NX,)),
            pltpu.SemaphoreType.DMA((1,)),
            pltpu.SemaphoreType.DMA((NG, 3)),
            pltpu.SemaphoreType.DMA((NG, 3)),
            pltpu.SemaphoreType.DMA((2,)),
            pltpu.SemaphoreType.DMA((2,)),
        ],
        compiler_params=pltpu.CompilerParams(
            dimension_semantics=("arbitrary",),
            vmem_limit_bytes=120 * 1024 * 1024,
            flags={f: True for f in _os.environ.get("K_FLAGS", "").split(",") if f},
        ),
    )(x, c, A_w_q, A_w_uk, A_w_uv, B_wqkv, gw, wo, B_wo)
    return out.reshape(1, S, M)
```

```python
import functools
import math
import os as _os

import jax
import jax.numpy as jnp
from jax import lax
import jax.experimental.pallas as pl
import jax.experimental.pallas.tpu as pltpu

S = 2048
M = 1024
H = 32
D = 128
DC = 512
DH = 32
W_B = 8
DIL = 2
KCAT = H * D + M

BQ = 256
HQ = BQ // 2
TK = int(_os.environ.get("K_TK", "256"))
RP = int(_os.environ.get("K_RP", "32"))
FB = int(_os.environ.get("K_FB", "3"))
BT0 = int(_os.environ.get("K_BT0", "1"))
RL = tuple(int(t) for t in _os.environ.get("K_RL", "0,16,0").split(","))
TLAG = int(_os.environ.get("K_TLAG", "2"))
F0 = int(_os.environ.get("K_F0", "2"))
F1 = int(_os.environ.get("K_F1", "2"))
LEAD = int(_os.environ.get("K_LEAD", "2"))
HG = 8
NG = H // HG
CH = S // HG
NX = 4
XR = S // NX
OUT_ROWS = int(_os.environ.get("K_OR", "128"))
N_OUT = S // OUT_ROWS
LOG2E = math.log2(math.e)
NEG = -1e9

_NT = (((1,), (1,)), ((), ()))
_TT = (((0,), (1,)), ((), ()))


def _drain(gen):
    for _ in gen:
        pass


def _fold(s, op):
    return functools.reduce(op, [s[:, c0:c0 + 128] for c0 in range(0, s.shape[1], 128)])


def _tied(a, tie):
    if tie is None:
        return a
    never, t = tie
    first = jnp.where(never, t[0:16, 0:128].astype(a.dtype), a[0:16, 0:128])
    return jnp.concatenate([jnp.concatenate([first, a[0:16, 128:]], axis=1), a[16:]], axis=0)


def _proj(x_ref, c_ref, wq_s, wuk_s, wuv_s, q_ref, k_ref, v_ref, h, slot):
    tie = yield
    for w_s, o_ref in ((wuk_s, k_ref), (wuv_s, v_ref)):
        for r in range(2):
            rows = pl.ds(r * (S // 2), S // 2)
            o_ref[slot, rows, :] = jnp.dot(_tied(c_ref[rows, :], tie), w_s[h],
                                           preferred_element_type=jnp.float32
                                           ).astype(jnp.bfloat16)
            tie = yield True
    for r in range(4):
        rows = pl.ds(r * (S // 4), S // 4)
        q = jnp.dot(_tied(x_ref[rows, :], tie), wq_s[h], preferred_element_type=jnp.float32)
        q_ref[slot, rows, :] = (q * (LOG2E * D ** -0.5)).astype(jnp.bfloat16)
        tie = yield True


def _attn_a(q_ref, k_ref, v_ref, g_ref, cat_ref, slot, hcol, never, filler, side):
    nq = S // BQ
    row = lax.broadcasted_iota(jnp.int32, (BQ, HQ), 0)
    col = lax.broadcasted_iota(jnp.int32, (BQ, HQ), 1)
    mask_a = col <= row
    mask_b = mask_a[:HQ]
    finals = {}

    def qk_block(i):
        lo = i * BQ
        q = q_ref[slot, pl.ds(lo, BQ), :]
        ss, mx = [], None
        for s0 in range(0, lo, TK):
            s = lax.dot_general(q, k_ref[slot, pl.ds(s0, min(TK, lo - s0)), :], _NT,
                                preferred_element_type=jnp.float32)
            ss.append(s)
            f = _fold(s, jnp.maximum)
            mx = f if mx is None else jnp.maximum(mx, f)
            yield None
        sa = lax.dot_general(q, k_ref[slot, pl.ds(lo, HQ), :], _NT,
                             preferred_element_type=jnp.float32)
        sa = jnp.where(mask_a, sa, NEG)
        sb = lax.dot_general(q[HQ:], k_ref[slot, pl.ds(lo + HQ, HQ), :], _NT,
                             preferred_element_type=jnp.float32)
        sb = jnp.where(mask_b, sb, NEG)
        mx = sa if mx is None else jnp.maximum(mx, sa)
        mx = jnp.concatenate([mx[:HQ], jnp.maximum(mx[HQ:], sb)], axis=0)
        m = jnp.broadcast_to(jnp.max(mx, axis=1, keepdims=True), (BQ, 128))
        yield ss, sa, sb, m

    def pv_block(i, ss, sa, sb, m, last=False):
        lo = i * BQ
        if i - TLAG in finals:
            m = jnp.where(never, finals[i - TLAG], m)
        lsum, o, ps = None, None, []
        for s in ss:
            p = jnp.exp2(s - jnp.concatenate([m] * (s.shape[1] // 128), axis=1))
            f = _fold(p, jnp.add)
            lsum = f if lsum is None else lsum + f
            ps.append(p.astype(jnp.bfloat16))
        if last:
            fill(F1, lsum)
        for t, p in enumerate(ps):
            d = jnp.dot(p, v_ref[slot, pl.ds(t * TK, p.shape[1]), :],
                        preferred_element_type=jnp.float32)
            o = d if o is None else o + d
            yield
        pa = jnp.exp2(sa - m)
        d = jnp.dot(pa.astype(jnp.bfloat16), v_ref[slot, pl.ds(lo, HQ), :],
                    preferred_element_type=jnp.float32)
        o = d if o is None else o + d
        lsum = pa if lsum is None else lsum + pa
        pb = jnp.exp2(sb - m[HQ:])
        d = jnp.dot(pb.astype(jnp.bfloat16), v_ref[slot, pl.ds(lo + HQ, HQ), :],
                    preferred_element_type=jnp.float32)
        o = jnp.concatenate([o[:HQ], o[HQ:] + d], axis=0)
        lsum = jnp.concatenate([lsum[:HQ], lsum[HQ:] + pb], axis=0)
        l = jnp.sum(lsum, axis=1, keepdims=True)
        r = pl.reciprocal(l, approx=True)
        r = r * (2.0 - l * r)
        o = o * (g_ref[pl.ds(lo, BQ), :] * r)
        finals[i] = o
        cat_ref[pl.ds(lo, BQ), pl.ds(hcol, D)] = o.astype(jnp.bfloat16)
        yield

    left = [8 if filler is not None else 0]

    def fill(n, tie=None):
        for k in range(n):
            if left[0] > 0:
                left[0] -= 1
                filler.send((never, tie) if (tie is not None and k == n - 1) else None)

    cur = next(qk_block(0))
    fill(F0)
    for i in range(nq - 1):
        pv, nxt = pv_block(i, *cur), qk_block(i + 1)
        for _ in range(LEAD):
            r = next(nxt)
            if r is not None:
                break
        while r is None:
            next(pv, None)
            r = next(nxt)
        cur = r
        _drain(pv)
    _drain(pv_block(nq - 1, *cur, last=True))
    fill(left[0] - FB)
    tie = next(side)
    fill(1, tie if BT0 else None)
    fill(left[0] - 1)
    fill(1, next(side))


def _attn_b(bt_ref, ot_ref, g_ref, cat_ref, h):
    c0 = pl.multiple_of((h % HG) * CH, CH)
    pos = c0 + lax.broadcasted_iota(jnp.int32, (HG, CH), 1)

    def taps(j, d):
        win = bt_ref[j, d, :, pl.ds(c0, CH + 128)]
        return [win[:, 128:] if w == 0 else pltpu.roll(win, w * DIL, 1)[:, 128:]
                for w in range(W_B)]

    logits = [None] * W_B
    for d in range(DH):
        qd = bt_ref[0, d, :, pl.ds(c0 + 128, CH)]
        for w, kw in enumerate(taps(1, d)):
            logits[w] = qd * kw if d == 0 else logits[w] + qd * kw
    logits = [l * (LOG2E * DH ** -0.5) for l in logits]
    logits = [l if w == 0 else jnp.where(pos >= w * DIL, l, NEG) for w, l in enumerate(logits)]
    mb = functools.reduce(jnp.maximum, logits)
    ps = [jnp.exp2(l - mb) for l in logits]
    inv = 1.0 / functools.reduce(lambda a, b: a + b, ps)
    ps = [p * inv for p in ps]
    tie = functools.reduce(jnp.add, ps)
    yield jnp.concatenate([tie[:, :128], tie[:, 128:]], axis=0)
    for d in range(DH):
        acc = None
        for w, vw in enumerate(taps(2, d)):
            acc = ps[w] * vw if w == 0 else acc + ps[w] * vw
        ot_ref[d] = acc
    o = jnp.swapaxes(ot_ref[...], 0, 1).reshape(HG * DH, CH)
    gi = 1.0 - g_ref[pl.ds(c0, CH), :]
    bcol = pl.multiple_of(H * D + (h // HG) * (HG * DH), HG * DH)
    for j in range(HG * DH // 128):
        oj = o[j * 128:(j + 1) * 128, :].T * gi
        cat_ref[pl.ds(c0, CH), pl.ds(bcol + j * 128, 128)] = oj.astype(jnp.bfloat16)
        tie = oj[0:16] + oj[CH - 16:] if j == 0 else tie + oj[0:16] + oj[CH - 16:]
    yield tie


def _kernel(x_hbm, c_hbm, wq_hbm, wuk_hbm, wuv_hbm, wb_hbm, gw_ref, wo_hbm, wob_hbm, out_hbm,
            x_s, c_s, wq_raw, wuk_raw, wuv_raw, wq_s, wuk_s, wuv_s, wb_s, cat_ref, wcat_ref,
            g_ref, q_ref, k_ref, v_ref, bt_ref, ot_ref, ostage, sem_x, sem_c, sem_a, sem_b, sem_o,
            sem_out):
    def x_copy(i):
        rows = pl.ds(i * XR, XR)
        return pltpu.make_async_copy(x_hbm.at[rows, :], x_s.at[rows, :], sem_x.at[i])

    def c_copy():
        return pltpu.make_async_copy(c_hbm, c_s, sem_c.at[0])

    def a_copies(g):
        hs = pl.ds(g * HG, HG)
        return [pltpu.make_async_copy(src.at[:, hs, :], dst.at[g], sem_a.at[g, j])
                for j, (src, dst) in enumerate(((wq_hbm, wq_raw), (wuk_hbm, wuk_raw),
                                                (wuv_hbm, wuv_raw)))]

    def b_copies(g):
        return [pltpu.make_async_copy(
            wb_hbm.at[:, pl.ds(pl.multiple_of(j * M + g * (HG * DH), HG * DH), HG * DH)],
            wb_s.at[j, g], sem_b.at[g, j]) for j in range(3)]

    def o_copies():
        return [pltpu.make_async_copy(wo_hbm, wcat_ref.at[pl.ds(0, H * D), :], sem_o.at[0]),
                pltpu.make_async_copy(wob_hbm, wcat_ref.at[pl.ds(H * D, M), :], sem_o.at[1])]

    def out_copy(r, slot):
        return pltpu.make_async_copy(
            ostage.at[slot], out_hbm.at[pl.ds(pl.multiple_of(r * OUT_ROWS, OUT_ROWS), OUT_ROWS), :],
            sem_out.at[slot])

    def start(cps):
        for cp in cps:
            cp.start()

    def wait(cps):
        for cp in cps:
            cp.wait()

    def relayout(g, i, n):
        ties = []
        for raw, dst in ((wq_raw, wq_s), (wuk_raw, wuk_s), (wuv_raw, wuv_s)):
            rows = dst.shape[1] // n
            for r in range(0, rows, RP):
                r0 = pl.multiple_of(i * rows + r, RP)
                v = jnp.swapaxes(raw[g, pl.ds(r0, RP)], 0, 1)
                dst[pl.ds(g * HG, HG), pl.ds(r0, RP), :] = v
                ties.append(functools.reduce(jnp.maximum, [
                    v[hh, rr:rr + 16] for hh in range(HG) for rr in range(0, RP, 16)]))
        return ties

    def b_proj(g, first):
        def body(i, carry):
            if first:
                x_copy(i).wait()

                @pl.when(i == 0)
                def _():
                    start([x_copy(j) for j in range(1, NX)])

                @pl.when(i == 1)
                def _():
                    start([c_copy()] + a_copies(0))

                @pl.when(i == 2)
                def _():
                    start(a_copies(1))

                @pl.when(i == 3)
                def _():
                    start(b_copies(1))
            x = x_s[pl.ds(pl.multiple_of(i * XR, XR), XR), :]
            ties = [] if first else relayout(jnp.minimum(g + 1, NG - 1), i, NX)
            for j in range(3):
                n = min(RL[j], len(ties))
                xj = _tied(x, (i < 0, functools.reduce(
                    jnp.maximum, [ties.pop() for _ in range(n)])) if n else None)
                t = lax.dot_general(wb_s[j, g], xj, _TT, preferred_element_type=jnp.float32)
                bt_ref[j, :, :, pl.ds(pl.multiple_of(128 + i * XR, 128), XR)] = jnp.swapaxes(
                    t.reshape(HG, DH, XR), 0, 1)
            return carry
        lax.fori_loop(0, NX, body, 0)

    x_copy(0).start()
    start(b_copies(0))
    bt_ref[:, :, :, pl.ds(0, 128)] = jnp.zeros((3, DH, HG, 128), jnp.float32)
    wait(b_copies(0))
    b_proj(0, True)
    wait([c_copy()] + a_copies(0) + a_copies(1))
    start(o_copies())
    never0 = pl.program_id(0) < 0
    tie = functools.reduce(jnp.maximum, relayout(0, 0, 1))
    gw = _tied(jnp.broadcast_to(gw_ref[...], (32, M)), (never0, tie))[0:16]
    z = lax.dot_general(gw, x_s[...], _NT, preferred_element_type=jnp.float32)
    gt = jax.nn.sigmoid(z[0:8])
    gt = jnp.concatenate([gt] * 16, axis=0)
    for r in range(S // 128):
        g_ref[pl.ds(r * 128, 128), :] = gt[:, r * 128:(r + 1) * 128].T
    p0 = _proj(x_s, c_s, wq_s, wuk_s, wuv_s, q_ref, k_ref, v_ref, 0, 0)
    next(p0)
    ties = relayout(1, 0, 1)
    for k in range(8):
        n = len(ties) // (8 - k)
        p0.send((never0, functools.reduce(jnp.maximum, [ties.pop() for _ in range(n)])))

    def head(h, nxt):
        never = h < 0
        slot = h % 2
        side = _attn_b(bt_ref, ot_ref, g_ref, cat_ref, h)
        filler = None
        if nxt:
            filler = _proj(x_s, c_s, wq_s, wuk_s, wuv_s, q_ref, k_ref, v_ref, h + 1, 1 - slot)
            next(filler)
        _attn_a(q_ref, k_ref, v_ref, g_ref, cat_ref, slot, pl.multiple_of(h * D, D),
                never, filler, side)
        _drain(side)

    def group_body(g, carry):
        @pl.when(g > 0)
        def _():
            wait(b_copies(g))

            @pl.when(g + 1 < NG)
            def _():
                wait(a_copies(g + 1))
            b_proj(g, False)

        @pl.when(g + 2 < NG)
        def _():
            start(a_copies(g + 2))

        @pl.when(jnp.logical_and(g > 0, g + 1 < NG))
        def _():
            start(b_copies(g + 1))

        def head_body(hl, carry):
            head(g * HG + hl, True)
            return carry
        lax.fori_loop(0, jnp.where(g == NG - 1, HG - 1, HG), head_body, 0)
        return carry

    lax.fori_loop(0, NG, group_body, 0)
    head(pl.program_id(0) + (H - 1), False)

    wait(o_copies())

    def out_body(r, carry):
        slot = r % 2

        @pl.when(r >= 2)
        def _():
            out_copy(r - 2, slot).wait()
        rows = pl.ds(pl.multiple_of(r * OUT_ROWS, OUT_ROWS), OUT_ROWS)
        ostage[slot] = jnp.dot(cat_ref[rows, :], wcat_ref[...],
                               preferred_element_type=jnp.float32).astype(ostage.dtype)
        out_copy(r, slot).start()
        return carry

    lax.fori_loop(0, N_OUT, out_body, 0)
    out_copy(N_OUT - 2, 0).wait()
    out_copy(N_OUT - 1, 1).wait()


@jax.jit
def pallas_gated_mix__compressed_kv_cla__sliding_local_dilated__prompt_kernel(
    A_x: jax.Array,
    A_c_kv: jax.Array,
    A_w_q: jax.Array,
    A_w_uk: jax.Array,
    A_w_uv: jax.Array,
    A_w_o: jax.Array,
    B_x: jax.Array,
    B_wqkv: jax.Array,
    B_wo: jax.Array,
    gate_w: jax.Array,
):
    del B_x
    x = A_x.reshape(S, M)
    c = A_c_kv.reshape(S, DC)
    wo = A_w_o.reshape(H * D, M)
    gw = gate_w.reshape(1, M)
    bf = jnp.bfloat16
    hbm = pl.BlockSpec(memory_space=pl.ANY)
    out = pl.pallas_call(
        _kernel,
        grid=(1,),
        in_specs=[hbm, hbm, hbm, hbm, hbm, hbm,
                  pl.BlockSpec((1, M), lambda s: (0, 0)), hbm, hbm],
        out_specs=hbm,
        out_shape=jax.ShapeDtypeStruct((S, M), bf),
        scratch_shapes=[
            pltpu.VMEM((S, M), bf),
            pltpu.VMEM((S, DC), bf),
            pltpu.VMEM((NG, M, HG, D), bf),
            pltpu.VMEM((NG, DC, HG, D), bf),
            pltpu.VMEM((NG, DC, HG, D), bf),
            pltpu.VMEM((H, M, D), bf),
            pltpu.VMEM((H, DC, D), bf),
            pltpu.VMEM((H, DC, D), bf),
            pltpu.VMEM((3, NG, M, HG * DH), bf),
            pltpu.VMEM((S, KCAT), bf),
            pltpu.VMEM((KCAT, M), bf),
            pltpu.VMEM((S, 128), jnp.float32),
            pltpu.VMEM((2, S, D), bf),
            pltpu.VMEM((2, S, D), bf),
            pltpu.VMEM((2, S, D), bf),
            pltpu.VMEM((3, DH, HG, 128 + S), jnp.float32),
            pltpu.VMEM((DH, HG, CH), jnp.float32),
            pltpu.VMEM((2, OUT_ROWS, M), bf),
            pltpu.SemaphoreType.DMA((NX,)),
            pltpu.SemaphoreType.DMA((1,)),
            pltpu.SemaphoreType.DMA((NG, 3)),
            pltpu.SemaphoreType.DMA((NG, 3)),
            pltpu.SemaphoreType.DMA((2,)),
            pltpu.SemaphoreType.DMA((2,)),
        ],
        compiler_params=pltpu.CompilerParams(
            dimension_semantics=("arbitrary",),
            vmem_limit_bytes=120 * 1024 * 1024,
            flags={f: True for f in _os.environ.get("K_FLAGS", "").split(",") if f},
        ),
    )(x, c, A_w_q, A_w_uk, A_w_uv, B_wqkv, gw, wo, B_wo)
    return out.reshape(1, S, M)
```

```python
import functools
import math

import jax
import jax.numpy as jnp
from jax import lax
import jax.experimental.pallas as pl
import jax.experimental.pallas.tpu as pltpu

S = 2048
M = 1024
H = 32
D = 128
DC = 512
DH = 32
W_B = 8
DIL = 2
KCAT = H * D + M

BQ = 256
HQ = BQ // 2
TK = 256
LEAD = 2
TLAG = 3
F0, F1, FB = 2, 2, 3
RP = 16
OUT_ROWS = 128
HG = 8
NG = H // HG
CH = S // HG
NX = 4
XR = S // NX
N_OUT = S // OUT_ROWS
LOG2E = math.log2(math.e)
NEG = -1e9

_NT = (((1,), (1,)), ((), ()))
_TT = (((0,), (1,)), ((), ()))


def _drain(gen):
    for _ in gen:
        pass


def _fold(s, op):
    return functools.reduce(op, [s[:, c0:c0 + 128] for c0 in range(0, s.shape[1], 128)])


def _tied(a, tie):
    if tie is None:
        return a
    never, t = tie
    first = jnp.where(never, t[0:16, 0:128].astype(a.dtype), a[0:16, 0:128])
    return jnp.concatenate([jnp.concatenate([first, a[0:16, 128:]], axis=1), a[16:]], axis=0)


def _proj(x_ref, c_ref, wq_s, wuk_s, wuv_s, q_ref, k_ref, v_ref, h, slot):
    tie = yield
    for w_s, o_ref in ((wuk_s, k_ref), (wuv_s, v_ref)):
        for r in range(2):
            rows = pl.ds(r * (S // 2), S // 2)
            o_ref[slot, rows, :] = jnp.dot(_tied(c_ref[rows, :], tie), w_s[h],
                                           preferred_element_type=jnp.float32
                                           ).astype(jnp.bfloat16)
            tie = yield True
    for r in range(4):
        rows = pl.ds(r * (S // 4), S // 4)
        q = jnp.dot(_tied(x_ref[rows, :], tie), wq_s[h], preferred_element_type=jnp.float32)
        q_ref[slot, rows, :] = (q * (LOG2E * D ** -0.5)).astype(jnp.bfloat16)
        tie = yield True


def _attn_a(q_ref, k_ref, v_ref, g_ref, cat_ref, slot, hcol, never, filler, side):
    nq = S // BQ
    row = lax.broadcasted_iota(jnp.int32, (BQ, HQ), 0)
    col = lax.broadcasted_iota(jnp.int32, (BQ, HQ), 1)
    mask_a = col <= row
    mask_b = mask_a[:HQ]
    finals = {}

    def qk_block(i):
        lo = i * BQ
        q = q_ref[slot, pl.ds(lo, BQ), :]
        ss, mx = [], None
        for s0 in range(0, lo, TK):
            s = lax.dot_general(q, k_ref[slot, pl.ds(s0, min(TK, lo - s0)), :], _NT,
                                preferred_element_type=jnp.float32)
            ss.append(s)
            f = _fold(s, jnp.maximum)
            mx = f if mx is None else jnp.maximum(mx, f)
            yield None
        sa = lax.dot_general(q, k_ref[slot, pl.ds(lo, HQ), :], _NT,
                             preferred_element_type=jnp.float32)
        sa = jnp.where(mask_a, sa, NEG)
        sb = lax.dot_general(q[HQ:], k_ref[slot, pl.ds(lo + HQ, HQ), :], _NT,
                             preferred_element_type=jnp.float32)
        sb = jnp.where(mask_b, sb, NEG)
        mx = sa if mx is None else jnp.maximum(mx, sa)
        mx = jnp.concatenate([mx[:HQ], jnp.maximum(mx[HQ:], sb)], axis=0)
        m = jnp.broadcast_to(jnp.max(mx, axis=1, keepdims=True), (BQ, 128))
        yield ss, sa, sb, m

    def pv_block(i, ss, sa, sb, m, last=False):
        lo = i * BQ
        if i - TLAG in finals:
            m = jnp.where(never, finals[i - TLAG], m)
        lsum, o, ps = None, None, []
        for s in ss:
            p = jnp.exp2(s - jnp.concatenate([m] * (s.shape[1] // 128), axis=1))
            f = _fold(p, jnp.add)
            lsum = f if lsum is None else lsum + f
            ps.append(p.astype(jnp.bfloat16))
        if last:
            fill(F1, lsum)
        for t, p in enumerate(ps):
            d = jnp.dot(p, v_ref[slot, pl.ds(t * TK, p.shape[1]), :],
                        preferred_element_type=jnp.float32)
            o = d if o is None else o + d
            yield
        pa = jnp.exp2(sa - m)
        d = jnp.dot(pa.astype(jnp.bfloat16), v_ref[slot, pl.ds(lo, HQ), :],
                    preferred_element_type=jnp.float32)
        o = d if o is None else o + d
        lsum = pa if lsum is None else lsum + pa
        pb = jnp.exp2(sb - m[HQ:])
        d = jnp.dot(pb.astype(jnp.bfloat16), v_ref[slot, pl.ds(lo + HQ, HQ), :],
                    preferred_element_type=jnp.float32)
        o = jnp.concatenate([o[:HQ], o[HQ:] + d], axis=0)
        lsum = jnp.concatenate([lsum[:HQ], lsum[HQ:] + pb], axis=0)
        l = jnp.sum(lsum, axis=1, keepdims=True)
        r = pl.reciprocal(l, approx=True)
        r = r * (2.0 - l * r)
        o = o * (g_ref[pl.ds(lo, BQ), :] * r)
        finals[i] = o
        cat_ref[pl.ds(lo, BQ), pl.ds(hcol, D)] = o.astype(jnp.bfloat16)
        yield

    left = [8 if filler is not None else 0]

    def fill(n, tie=None):
        for k in range(n):
            if left[0] > 0:
                left[0] -= 1
                filler.send((never, tie) if (tie is not None and k == n - 1) else None)

    cur = next(qk_block(0))
    fill(F0)
    for i in range(nq - 1):
        pv, nxt = pv_block(i, *cur), qk_block(i + 1)
        for _ in range(LEAD):
            r = next(nxt)
            if r is not None:
                break
        while r is None:
            next(pv, None)
            r = next(nxt)
        cur = r
        _drain(pv)
    _drain(pv_block(nq - 1, *cur, last=True))
    fill(left[0] - FB)
    tie = next(side)
    fill(1, tie)
    fill(left[0] - 1)
    fill(1, next(side))


def _attn_b(bt_ref, ot_ref, g_ref, cat_ref, h):
    c0 = pl.multiple_of((h % HG) * CH, CH)
    pos = c0 + lax.broadcasted_iota(jnp.int32, (HG, CH), 1)

    def taps(j, d):
        win = bt_ref[j, d, :, pl.ds(c0, CH + 128)]
        return [win[:, 128:] if w == 0 else pltpu.roll(win, w * DIL, 1)[:, 128:]
                for w in range(W_B)]

    logits = [None] * W_B
    for d in range(DH):
        qd = bt_ref[0, d, :, pl.ds(c0 + 128, CH)]
        for w, kw in enumerate(taps(1, d)):
            logits[w] = qd * kw if d == 0 else logits[w] + qd * kw
    logits = [l * (LOG2E * DH ** -0.5) for l in logits]
    logits = [l if w == 0 else jnp.where(pos >= w * DIL, l, NEG) for w, l in enumerate(logits)]
    mb = functools.reduce(jnp.maximum, logits)
    ps = [jnp.exp2(l - mb) for l in logits]
    inv = 1.0 / functools.reduce(lambda a, b: a + b, ps)
    ps = [p * inv for p in ps]
    tie = functools.reduce(jnp.add, ps)
    yield jnp.concatenate([tie[:, :128], tie[:, 128:]], axis=0)
    for d in range(DH):
        acc = None
        for w, vw in enumerate(taps(2, d)):
            acc = ps[w] * vw if w == 0 else acc + ps[w] * vw
        ot_ref[d] = acc
    o = jnp.swapaxes(ot_ref[...], 0, 1).reshape(HG * DH, CH)
    gi = 1.0 - g_ref[pl.ds(c0, CH), :]
    bcol = pl.multiple_of(H * D + (h // HG) * (HG * DH), HG * DH)
    for j in range(HG * DH // 128):
        oj = o[j * 128:(j + 1) * 128, :].T * gi
        cat_ref[pl.ds(c0, CH), pl.ds(bcol + j * 128, 128)] = oj.astype(jnp.bfloat16)
        tie = oj[0:16] + oj[CH - 16:] if j == 0 else tie + oj[0:16] + oj[CH - 16:]
    yield tie


def _kernel(x_hbm, c_hbm, wq_hbm, wuk_hbm, wuv_hbm, wb_hbm, gw_ref, wo_hbm, wob_hbm, out_hbm,
            x_s, c_s, wq_raw, wuk_raw, wuv_raw, wq_s, wuk_s, wuv_s, wb_s, cat_ref, wcat_ref,
            g_ref, q_ref, k_ref, v_ref, bt_ref, ot_ref, ostage, sem_x, sem_c, sem_a, sem_b, sem_o,
            sem_out):
    def x_copy(i):
        rows = pl.ds(i * XR, XR)
        return pltpu.make_async_copy(x_hbm.at[rows, :], x_s.at[rows, :], sem_x.at[i])

    def c_copy():
        return pltpu.make_async_copy(c_hbm, c_s, sem_c.at[0])

    def a_copies(g):
        hs = pl.ds(g * HG, HG)
        return [pltpu.make_async_copy(src.at[:, hs, :], dst.at[g], sem_a.at[g, j])
                for j, (src, dst) in enumerate(((wq_hbm, wq_raw), (wuk_hbm, wuk_raw),
                                                (wuv_hbm, wuv_raw)))]

    def b_copies(g):
        return [pltpu.make_async_copy(
            wb_hbm.at[:, pl.ds(pl.multiple_of(j * M + g * (HG * DH), HG * DH), HG * DH)],
            wb_s.at[j, g], sem_b.at[g, j]) for j in range(3)]

    def o_copies():
        return [pltpu.make_async_copy(wo_hbm, wcat_ref.at[pl.ds(0, H * D), :], sem_o.at[0]),
                pltpu.make_async_copy(wob_hbm, wcat_ref.at[pl.ds(H * D, M), :], sem_o.at[1])]

    def out_copy(r, slot):
        return pltpu.make_async_copy(
            ostage.at[slot], out_hbm.at[pl.ds(pl.multiple_of(r * OUT_ROWS, OUT_ROWS), OUT_ROWS), :],
            sem_out.at[slot])

    def start(cps):
        for cp in cps:
            cp.start()

    def wait(cps):
        for cp in cps:
            cp.wait()

    def relayout(g, i, n, never):
        ties = []
        for raw, dst in ((wq_raw, wq_s), (wuk_raw, wuk_s), (wuv_raw, wuv_s)):
            rows = dst.shape[1] // n
            for r in range(0, rows, RP):
                r0 = pl.multiple_of(i * rows + r, RP)
                u = raw[g, pl.ds(r0, RP)]
                if ties:
                    u = jnp.concatenate([
                        x for r1 in range(0, RP, 16) for x in (
                            jnp.where(never, ties[-1][0:8], u[r1])[None], u[r1 + 1:r1 + 16])], 0)
                v = jnp.swapaxes(u, 0, 1)
                dst[pl.ds(g * HG, HG), pl.ds(r0, RP), :] = v
                ties.append(functools.reduce(jnp.maximum, [
                    v[hh, rr:rr + 16] for hh in range(HG) for rr in range(0, RP, 16)]))
        return ties

    def b_proj(g, first):
        def body(i, carry):
            if first:
                x_copy(i).wait()

                @pl.when(i == 0)
                def _():
                    start([x_copy(j) for j in range(1, NX)])

                @pl.when(i == 1)
                def _():
                    start([c_copy()] + a_copies(0))

                @pl.when(i == 2)
                def _():
                    start(a_copies(1))

                @pl.when(i == 3)
                def _():
                    start(b_copies(1))
            x = x_s[pl.ds(pl.multiple_of(i * XR, XR), XR), :]
            ties = [] if first else relayout(jnp.minimum(g + 1, NG - 1), i, NX, i < 0)
            nt = len(ties)
            for j in range(3):
                n = 0 if j == 0 else nt // 2
                xj = _tied(x, (i < 0, functools.reduce(
                    jnp.maximum, [ties.pop() for _ in range(n)])) if n else None)
                t = lax.dot_general(wb_s[j, g], xj, _TT, preferred_element_type=jnp.float32)
                bt_ref[j, :, :, pl.ds(pl.multiple_of(128 + i * XR, 128), XR)] = jnp.swapaxes(
                    t.reshape(HG, DH, XR), 0, 1)
            return carry
        lax.fori_loop(0, NX, body, 0)

    x_copy(0).start()
    start(b_copies(0))
    bt_ref[:, :, :, pl.ds(0, 128)] = jnp.zeros((3, DH, HG, 128), jnp.float32)
    wait(b_copies(0))
    b_proj(0, True)
    wait([c_copy()] + a_copies(0) + a_copies(1))
    start(o_copies())
    never0 = pl.program_id(0) < 0
    tie = functools.reduce(jnp.maximum, relayout(0, 0, 1, never0))
    gw = _tied(jnp.broadcast_to(gw_ref[...].reshape(1, M), (32, M)), (never0, tie))[0:16]
    z = lax.dot_general(gw, x_s[...], _NT, preferred_element_type=jnp.float32)
    gt = jax.nn.sigmoid(z[0:8])
    gt = jnp.concatenate([gt] * 16, axis=0)
    for r in range(S // 128):
        g_ref[pl.ds(r * 128, 128), :] = gt[:, r * 128:(r + 1) * 128].T
    p0 = _proj(x_s, c_s, wq_s, wuk_s, wuv_s, q_ref, k_ref, v_ref, 0, 0)
    next(p0)
    ties = relayout(1, 0, 1, never0)
    for k in range(8):
        n = len(ties) // (8 - k)
        p0.send((never0, functools.reduce(jnp.maximum, [ties.pop() for _ in range(n)])))

    def head(h, nxt):
        never = h < 0
        slot = h % 2
        side = _attn_b(bt_ref, ot_ref, g_ref, cat_ref, h)
        filler = None
        if nxt:
            filler = _proj(x_s, c_s, wq_s, wuk_s, wuv_s, q_ref, k_ref, v_ref, h + 1, 1 - slot)
            next(filler)
        _attn_a(q_ref, k_ref, v_ref, g_ref, cat_ref, slot, pl.multiple_of(h * D, D),
                never, filler, side)
        _drain(side)

    def group_body(g, carry):
        @pl.when(g > 0)
        def _():
            wait(b_copies(g))

            @pl.when(g + 1 < NG)
            def _():
                wait(a_copies(g + 1))
            b_proj(g, False)

        @pl.when(g + 2 < NG)
        def _():
            start(a_copies(g + 2))

        @pl.when(jnp.logical_and(g > 0, g + 1 < NG))
        def _():
            start(b_copies(g + 1))

        def head_body(hl, carry):
            head(g * HG + hl, True)
            return carry
        lax.fori_loop(0, jnp.where(g == NG - 1, HG - 1, HG), head_body, 0)
        return carry

    lax.fori_loop(0, NG, group_body, 0)
    head(pl.program_id(0) + (H - 1), False)

    wait(o_copies())

    def out_body(r, carry):
        slot = r % 2

        @pl.when(r >= 2)
        def _():
            out_copy(r - 2, slot).wait()
        rows = pl.ds(pl.multiple_of(r * OUT_ROWS, OUT_ROWS), OUT_ROWS)
        ostage[slot] = jnp.dot(cat_ref[rows, :], wcat_ref[...],
                               preferred_element_type=jnp.float32).astype(ostage.dtype)
        out_copy(r, slot).start()
        return carry

    lax.fori_loop(0, N_OUT, out_body, 0)
    out_copy(N_OUT - 2, 0).wait()
    out_copy(N_OUT - 1, 1).wait()


@jax.jit
def pallas_gated_mix__compressed_kv_cla__sliding_local_dilated__prompt_kernel(
    A_x: jax.Array,
    A_c_kv: jax.Array,
    A_w_q: jax.Array,
    A_w_uk: jax.Array,
    A_w_uv: jax.Array,
    A_w_o: jax.Array,
    B_x: jax.Array,
    B_wqkv: jax.Array,
    B_wo: jax.Array,
    gate_w: jax.Array,
):
    del B_x
    x = A_x.reshape(S, M)
    c = A_c_kv.reshape(S, DC)
    wo = A_w_o.reshape(H * D, M)
    bf = jnp.bfloat16
    hbm = pl.BlockSpec(memory_space=pl.ANY)
    out = pl.pallas_call(
        _kernel,
        grid=(1,),
        in_specs=[hbm, hbm, hbm, hbm, hbm, hbm,
                  pl.BlockSpec((M,), lambda s: (0,)), hbm, hbm],
        out_specs=hbm,
        out_shape=jax.ShapeDtypeStruct((S, M), bf),
        scratch_shapes=[
            pltpu.VMEM((S, M), bf),
            pltpu.VMEM((S, DC), bf),
            pltpu.VMEM((NG, M, HG, D), bf),
            pltpu.VMEM((NG, DC, HG, D), bf),
            pltpu.VMEM((NG, DC, HG, D), bf),
            pltpu.VMEM((H, M, D), bf),
            pltpu.VMEM((H, DC, D), bf),
            pltpu.VMEM((H, DC, D), bf),
            pltpu.VMEM((3, NG, M, HG * DH), bf),
            pltpu.VMEM((S, KCAT), bf),
            pltpu.VMEM((KCAT, M), bf),
            pltpu.VMEM((S, 128), jnp.float32),
            pltpu.VMEM((2, S, D), bf),
            pltpu.VMEM((2, S, D), bf),
            pltpu.VMEM((2, S, D), bf),
            pltpu.VMEM((3, DH, HG, 128 + S), jnp.float32),
            pltpu.VMEM((DH, HG, CH), jnp.float32),
            pltpu.VMEM((2, OUT_ROWS, M), bf),
            pltpu.SemaphoreType.DMA((NX,)),
            pltpu.SemaphoreType.DMA((1,)),
            pltpu.SemaphoreType.DMA((NG, 3)),
            pltpu.SemaphoreType.DMA((NG, 3)),
            pltpu.SemaphoreType.DMA((2,)),
            pltpu.SemaphoreType.DMA((2,)),
        ],
        compiler_params=pltpu.CompilerParams(
            dimension_semantics=("arbitrary",),
            vmem_limit_bytes=120 * 1024 * 1024,
        ),
    )(x, c, A_w_q, A_w_uk, A_w_uv, B_wqkv, gate_w, wo, B_wo)
    return out.reshape(1, S, M)
```

```python
import functools
import math

import jax
import jax.numpy as jnp
from jax import lax
import jax.experimental.pallas as pl
import jax.experimental.pallas.tpu as pltpu

S = 2048
M = 1024
H = 32
D = 128
DC = 512
DH = 32
W_B = 8
DIL = 2
KCAT = H * D + M

BQ = 256
HQ = BQ // 2
TK = 256
LEAD = 2
TLAG = 2
F0, F1, FB = 2, 2, 3
RP = 16
OUT_ROWS = 128
HG = 8
NG = H // HG
CH = S // HG
NX = 4
XR = S // NX
N_OUT = S // OUT_ROWS
LOG2E = math.log2(math.e)
NEG = -1e9

_NT = (((1,), (1,)), ((), ()))
_TT = (((0,), (1,)), ((), ()))


def _drain(gen):
    for _ in gen:
        pass


def _fold(s, op):
    return functools.reduce(op, [s[:, c0:c0 + 128] for c0 in range(0, s.shape[1], 128)])


def _tied(a, tie):
    if tie is None:
        return a
    never, t = tie
    first = jnp.where(never, t[0:16, 0:128].astype(a.dtype), a[0:16, 0:128])
    return jnp.concatenate([jnp.concatenate([first, a[0:16, 128:]], axis=1), a[16:]], axis=0)


def _proj(x_ref, c_ref, wq_s, wuk_s, wuv_s, q_ref, k_ref, v_ref, h, slot):
    tie = yield
    for w_s, o_ref in ((wuk_s, k_ref), (wuv_s, v_ref)):
        for r in range(2):
            rows = pl.ds(r * (S // 2), S // 2)
            o_ref[slot, rows, :] = jnp.dot(_tied(c_ref[rows, :], tie), w_s[h],
                                           preferred_element_type=jnp.float32
                                           ).astype(jnp.bfloat16)
            tie = yield True
    for r in range(4):
        rows = pl.ds(r * (S // 4), S // 4)
        q = jnp.dot(_tied(x_ref[rows, :], tie), wq_s[h], preferred_element_type=jnp.float32)
        q_ref[slot, rows, :] = (q * (LOG2E * D ** -0.5)).astype(jnp.bfloat16)
        tie = yield True


def _attn_a(q_ref, k_ref, v_ref, g_ref, cat_ref, slot, hcol, never, filler, side):
    nq = S // BQ
    row = lax.broadcasted_iota(jnp.int32, (BQ, HQ), 0)
    col = lax.broadcasted_iota(jnp.int32, (BQ, HQ), 1)
    mask_a = col <= row
    mask_b = mask_a[:HQ]
    finals = {}

    def qk_block(i):
        lo = i * BQ
        q = q_ref[slot, pl.ds(lo, BQ), :]
        ss, mx = [], None
        for s0 in range(0, lo, TK):
            s = lax.dot_general(q, k_ref[slot, pl.ds(s0, min(TK, lo - s0)), :], _NT,
                                preferred_element_type=jnp.float32)
            ss.append(s)
            f = _fold(s, jnp.maximum)
            mx = f if mx is None else jnp.maximum(mx, f)
            yield None
        sa = lax.dot_general(q, k_ref[slot, pl.ds(lo, HQ), :], _NT,
                             preferred_element_type=jnp.float32)
        sa = jnp.where(mask_a, sa, NEG)
        sb = lax.dot_general(q[HQ:], k_ref[slot, pl.ds(lo + HQ, HQ), :], _NT,
                             preferred_element_type=jnp.float32)
        sb = jnp.where(mask_b, sb, NEG)
        mx = sa if mx is None else jnp.maximum(mx, sa)
        mx = jnp.concatenate([mx[:HQ], jnp.maximum(mx[HQ:], sb)], axis=0)
        m = jnp.broadcast_to(jnp.max(mx, axis=1, keepdims=True), (BQ, 128))
        yield ss, sa, sb, m

    def pv_block(i, ss, sa, sb, m, last=False):
        lo = i * BQ
        if i - TLAG in finals:
            m = jnp.where(never, finals[i - TLAG], m)
        lsum, o, ps = None, None, []
        for s in ss:
            p = jnp.exp2(s - jnp.concatenate([m] * (s.shape[1] // 128), axis=1))
            f = _fold(p, jnp.add)
            lsum = f if lsum is None else lsum + f
            ps.append(p.astype(jnp.bfloat16))
        if last:
            fill(F1, lsum)
        for t, p in enumerate(ps):
            d = jnp.dot(p, v_ref[slot, pl.ds(t * TK, p.shape[1]), :],
                        preferred_element_type=jnp.float32)
            o = d if o is None else o + d
            yield
        pa = jnp.exp2(sa - m)
        d = jnp.dot(pa.astype(jnp.bfloat16), v_ref[slot, pl.ds(lo, HQ), :],
                    preferred_element_type=jnp.float32)
        o = d if o is None else o + d
        lsum = pa if lsum is None else lsum + pa
        pb = jnp.exp2(sb - m[HQ:])
        d = jnp.dot(pb.astype(jnp.bfloat16), v_ref[slot, pl.ds(lo + HQ, HQ), :],
                    preferred_element_type=jnp.float32)
        o = jnp.concatenate([o[:HQ], o[HQ:] + d], axis=0)
        lsum = jnp.concatenate([lsum[:HQ], lsum[HQ:] + pb], axis=0)
        l = jnp.sum(lsum, axis=1, keepdims=True)
        r = pl.reciprocal(l, approx=True)
        r = r * (2.0 - l * r)
        o = o * (g_ref[pl.ds(lo, BQ), :] * r)
        finals[i] = o
        cat_ref[pl.ds(lo, BQ), pl.ds(hcol, D)] = o.astype(jnp.bfloat16)
        yield

    left = [8 if filler is not None else 0]

    def fill(n, tie=None):
        for k in range(n):
            if left[0] > 0:
                left[0] -= 1
                filler.send((never, tie) if (tie is not None and k == n - 1) else None)

    cur = next(qk_block(0))
    fill(F0)
    for i in range(nq - 1):
        pv, nxt = pv_block(i, *cur), qk_block(i + 1)
        for _ in range(LEAD):
            r = next(nxt)
            if r is not None:
                break
        while r is None:
            next(pv, None)
            r = next(nxt)
        cur = r
        _drain(pv)
    _drain(pv_block(nq - 1, *cur, last=True))
    fill(left[0] - FB)
    if side is not None:
        fill(1, next(side))
        fill(left[0] - 1)
        fill(1, next(side))


def _attn_b(bt_ref, ot_ref, g_ref, cat_ref, h):
    c0 = pl.multiple_of((h % HG) * CH, CH)
    pos = c0 + lax.broadcasted_iota(jnp.int32, (HG, CH), 1)

    def taps(j, d):
        win = bt_ref[j, d, :, pl.ds(c0, CH + 128)]
        return [win[:, 128:] if w == 0 else pltpu.roll(win, w * DIL, 1)[:, 128:]
                for w in range(W_B)]

    logits = [None] * W_B
    for d in range(DH):
        qd = bt_ref[0, d, :, pl.ds(c0 + 128, CH)]
        for w, kw in enumerate(taps(1, d)):
            logits[w] = qd * kw if d == 0 else logits[w] + qd * kw
    logits = [l * (LOG2E * DH ** -0.5) for l in logits]
    logits = [l if w == 0 else jnp.where(pos >= w * DIL, l, NEG) for w, l in enumerate(logits)]
    mb = functools.reduce(jnp.maximum, logits)
    ps = [jnp.exp2(l - mb) for l in logits]
    inv = 1.0 / functools.reduce(lambda a, b: a + b, ps)
    ps = [p * inv for p in ps]
    tie = functools.reduce(jnp.add, ps)
    yield jnp.concatenate([tie[:, :128], tie[:, 128:]], axis=0)
    for d in range(DH):
        acc = None
        for w, vw in enumerate(taps(2, d)):
            acc = ps[w] * vw if w == 0 else acc + ps[w] * vw
        ot_ref[d] = acc
    o = jnp.swapaxes(ot_ref[...], 0, 1).reshape(HG * DH, CH)
    gi = 1.0 - g_ref[pl.ds(c0, CH), :]
    bcol = pl.multiple_of(H * D + (h // HG) * (HG * DH), HG * DH)
    for j in range(HG * DH // 128):
        oj = o[j * 128:(j + 1) * 128, :].T * gi
        cat_ref[pl.ds(c0, CH), pl.ds(bcol + j * 128, 128)] = oj.astype(jnp.bfloat16)
        tie = oj[0:16] + oj[CH - 16:] if j == 0 else tie + oj[0:16] + oj[CH - 16:]
    yield tie


def _kernel(x_hbm, c_hbm, wq_hbm, wuk_hbm, wuv_hbm, wb_hbm, gw_ref, wo_hbm, wob_hbm, out_hbm,
            x_s, c_s, wq_raw, wuk_raw, wuv_raw, wq_s, wuk_s, wuv_s, wb_s, cat_ref, wcat_ref,
            g_ref, q_ref, k_ref, v_ref, bt_ref, ot_ref, ostage, sem_x, sem_c, sem_a, sem_b, sem_o,
            sem_out):
    def x_copy(i):
        rows = pl.ds(i * XR, XR)
        return pltpu.make_async_copy(x_hbm.at[rows, :], x_s.at[rows, :], sem_x.at[i])

    def c_copy():
        return pltpu.make_async_copy(c_hbm, c_s, sem_c.at[0])

    def a_copies(g):
        hs = pl.ds(g * HG, HG)
        return [pltpu.make_async_copy(src.at[:, hs, :], dst.at[g], sem_a.at[g, j])
                for j, (src, dst) in enumerate(((wq_hbm, wq_raw), (wuk_hbm, wuk_raw),
                                                (wuv_hbm, wuv_raw)))]

    def b_copies(g):
        return [pltpu.make_async_copy(
            wb_hbm.at[:, pl.ds(pl.multiple_of(j * M + g * (HG * DH), HG * DH), HG * DH)],
            wb_s.at[j, g], sem_b.at[g, j]) for j in range(3)]

    def o_copies():
        return [pltpu.make_async_copy(wo_hbm, wcat_ref.at[pl.ds(0, H * D), :], sem_o.at[0]),
                pltpu.make_async_copy(wob_hbm, wcat_ref.at[pl.ds(H * D, M), :], sem_o.at[1])]

    def out_copy(r, slot):
        return pltpu.make_async_copy(
            ostage.at[slot], out_hbm.at[pl.ds(pl.multiple_of(r * OUT_ROWS, OUT_ROWS), OUT_ROWS), :],
            sem_out.at[slot])

    def start(cps):
        for cp in cps:
            cp.start()

    def wait(cps):
        for cp in cps:
            cp.wait()

    def relayout(g, i, n, never):
        ties = []
        for raw, dst in ((wq_raw, wq_s), (wuk_raw, wuk_s), (wuv_raw, wuv_s)):
            rows = dst.shape[1] // n
            for r in range(0, rows, RP):
                r0 = pl.multiple_of(i * rows + r, RP)
                u = raw[g, pl.ds(r0, RP)]
                if ties:
                    u = jnp.concatenate([
                        x for r1 in range(0, RP, 16) for x in (
                            jnp.where(never, ties[-1][0:8], u[r1])[None], u[r1 + 1:r1 + 16])], 0)
                v = jnp.swapaxes(u, 0, 1)
                dst[pl.ds(g * HG, HG), pl.ds(r0, RP), :] = v
                ties.append(functools.reduce(jnp.maximum, [
                    v[hh, rr:rr + 16] for hh in range(HG) for rr in range(0, RP, 16)]))
        return ties

    def b_proj(g, first):
        def body(i, carry):
            if first:
                x_copy(i).wait()

                @pl.when(i == 0)
                def _():
                    start([x_copy(j) for j in range(1, NX)])

                @pl.when(i == 1)
                def _():
                    start([c_copy()] + a_copies(0))

                @pl.when(i == 2)
                def _():
                    start(a_copies(1))

                @pl.when(i == 3)
                def _():
                    start(b_copies(1))
            x = x_s[pl.ds(pl.multiple_of(i * XR, XR), XR), :]
            ties = [] if first else relayout(g, i, NX, i < 0)
            nt = len(ties)
            for j in range(3):
                n = 0 if j == 0 else nt // 2
                xj = _tied(x, (i < 0, functools.reduce(
                    jnp.maximum, [ties.pop() for _ in range(n)])) if n else None)
                t = lax.dot_general(wb_s[j, g], xj, _TT, preferred_element_type=jnp.float32)
                bt_ref[j, :, :, pl.ds(pl.multiple_of(128 + i * XR, 128), XR)] = jnp.swapaxes(
                    t.reshape(HG, DH, XR), 0, 1)
            return carry
        lax.fori_loop(0, NX, body, 0)

    x_copy(0).start()
    start(b_copies(0))
    bt_ref[:, :, :, pl.ds(0, 128)] = jnp.zeros((3, DH, HG, 128), jnp.float32)
    wait(b_copies(0))
    b_proj(0, True)
    wait([c_copy()] + a_copies(0))
    start(o_copies())
    never0 = pl.program_id(0) < 0
    tie = functools.reduce(jnp.maximum, relayout(0, 0, 1, never0))
    gw = _tied(jnp.broadcast_to(gw_ref[...].reshape(1, M), (32, M)), (never0, tie))[0:16]
    z = lax.dot_general(gw, x_s[...], _NT, preferred_element_type=jnp.float32)
    gt = jax.nn.sigmoid(z[0:8])
    gt = jnp.concatenate([gt] * 16, axis=0)
    for r in range(S // 128):
        g_ref[pl.ds(r * 128, 128), :] = gt[:, r * 128:(r + 1) * 128].T
    p0 = _proj(x_s, c_s, wq_s, wuk_s, wuv_s, q_ref, k_ref, v_ref, 0, 0)
    side0 = _attn_b(bt_ref, ot_ref, g_ref, cat_ref, pl.program_id(0))
    next(p0)
    for k in range(8):
        p0.send((never0, next(side0)) if k in (5, 7) else None)

    def head(h, nxt):
        never = h < 0
        slot = h % 2
        filler, side = None, None
        if nxt:
            filler = _proj(x_s, c_s, wq_s, wuk_s, wuv_s, q_ref, k_ref, v_ref, h + 1, 1 - slot)
            next(filler)
            side = _attn_b(bt_ref, ot_ref, g_ref, cat_ref, h + 1)
        _attn_a(q_ref, k_ref, v_ref, g_ref, cat_ref, slot, pl.multiple_of(h * D, D),
                never, filler, side)

    def group_body(g, carry):
        @pl.when(g > 0)
        def _():
            wait(b_copies(g) + a_copies(g))

            @pl.when(g + 1 < NG)
            def _():
                start(b_copies(g + 1) + a_copies(g + 1))
            b_proj(g, False)

        def head_body(hl, carry):
            head(g * HG + hl - 1, True)
            return carry
        lax.fori_loop(jnp.where(g == 0, 1, 0), HG, head_body, 0)
        return carry

    lax.fori_loop(0, NG, group_body, 0)
    head(pl.program_id(0) + (H - 1), False)

    wait(o_copies())

    def out_body(r, carry):
        slot = r % 2

        @pl.when(r >= 2)
        def _():
            out_copy(r - 2, slot).wait()
        rows = pl.ds(pl.multiple_of(r * OUT_ROWS, OUT_ROWS), OUT_ROWS)
        ostage[slot] = jnp.dot(cat_ref[rows, :], wcat_ref[...],
                               preferred_element_type=jnp.float32).astype(ostage.dtype)
        out_copy(r, slot).start()
        return carry

    lax.fori_loop(0, N_OUT, out_body, 0)
    out_copy(N_OUT - 2, 0).wait()
    out_copy(N_OUT - 1, 1).wait()


@jax.jit
def pallas_gated_mix__compressed_kv_cla__sliding_local_dilated__prompt_kernel(
    A_x: jax.Array,
    A_c_kv: jax.Array,
    A_w_q: jax.Array,
    A_w_uk: jax.Array,
    A_w_uv: jax.Array,
    A_w_o: jax.Array,
    B_x: jax.Array,
    B_wqkv: jax.Array,
    B_wo: jax.Array,
    gate_w: jax.Array,
):
    del B_x
    x = A_x.reshape(S, M)
    c = A_c_kv.reshape(S, DC)
    wo = A_w_o.reshape(H * D, M)
    bf = jnp.bfloat16
    hbm = pl.BlockSpec(memory_space=pl.ANY)
    out = pl.pallas_call(
        _kernel,
        grid=(1,),
        in_specs=[hbm, hbm, hbm, hbm, hbm, hbm,
                  pl.BlockSpec((M,), lambda s: (0,)), hbm, hbm],
        out_specs=hbm,
        out_shape=jax.ShapeDtypeStruct((S, M), bf),
        scratch_shapes=[
            pltpu.VMEM((S, M), bf),
            pltpu.VMEM((S, DC), bf),
            pltpu.VMEM((NG, M, HG, D), bf),
            pltpu.VMEM((NG, DC, HG, D), bf),
            pltpu.VMEM((NG, DC, HG, D), bf),
            pltpu.VMEM((H, M, D), bf),
            pltpu.VMEM((H, DC, D), bf),
            pltpu.VMEM((H, DC, D), bf),
            pltpu.VMEM((3, NG, M, HG * DH), bf),
            pltpu.VMEM((S, KCAT), bf),
            pltpu.VMEM((KCAT, M), bf),
            pltpu.VMEM((S, 128), jnp.float32),
            pltpu.VMEM((2, S, D), bf),
            pltpu.VMEM((2, S, D), bf),
            pltpu.VMEM((2, S, D), bf),
            pltpu.VMEM((3, DH, HG, 128 + S), jnp.float32),
            pltpu.VMEM((DH, HG, CH), jnp.float32),
            pltpu.VMEM((2, OUT_ROWS, M), bf),
            pltpu.SemaphoreType.DMA((NX,)),
            pltpu.SemaphoreType.DMA((1,)),
            pltpu.SemaphoreType.DMA((NG, 3)),
            pltpu.SemaphoreType.DMA((NG, 3)),
            pltpu.SemaphoreType.DMA((2,)),
            pltpu.SemaphoreType.DMA((2,)),
        ],
        compiler_params=pltpu.CompilerParams(
            dimension_semantics=("arbitrary",),
            vmem_limit_bytes=120 * 1024 * 1024,
        ),
    )(x, c, A_w_q, A_w_uk, A_w_uv, B_wqkv, gate_w, wo, B_wo)
    return out.reshape(1, S, M)
```
